```python
import os as _os
_os.environ.setdefault("JAX_PLATFORMS", "cpu")
import jax
import jax.numpy as jnp

def _softmax(x, axis=-1):
    return jax.nn.softmax(x, axis=axis)
def _gelu(x):
    return jax.nn.gelu(x, approximate=True)
def _silu(x):
    return jax.nn.silu(x)
def _sigmoid(x):
    return jax.nn.sigmoid(x)
def _layernorm(x, axis=-1, eps=1e-5):
    m = jnp.mean(x, axis=axis, keepdims=True)
    v = jnp.var(x, axis=axis, keepdims=True)
    return (x - m) / jnp.sqrt(v + eps)
def _scatter_add(tgt, idx, src, axis=0):
    return tgt.at[idx].add(src)
def _segment_sum(src, seg, n):
    return jax.ops.segment_sum(src, seg, n)
class _Rng:
    def __init__(self, key):
        self._k = key
    def _next(self):
        self._k, sub = jax.random.split(self._k)
        return sub
    def normal(self, shape):
        return jax.random.normal(self._next(), shape, dtype=jnp.bfloat16)
    def randint(self, lo, hi, shape):
        return jax.random.randint(self._next(), shape, lo, hi, dtype=jnp.int32)
    def uniform(self, shape, lo=0.0, hi=1.0):
        return jax.random.uniform(self._next(), shape, jnp.bfloat16, lo, hi)
    def permutation(self, n):
        return jax.random.permutation(self._next(), n)


kernel_name = 'interleave_layers__sliding_local_dilated__softmax_full_mha__prompt'

def setup_inputs():
    _rng = _Rng(jax.random.key(int.from_bytes(__import__("os").urandom(4), "little")))
    _w = (lambda a: (lambda t: t.astype(jnp.bfloat16) if jnp.issubdtype(t.dtype, jnp.floating) else t)(jnp.asarray(a)))
    def _A_setup():
        B, S, D = 1, 2048, 512
        return {
            "x": _w((lambda *s: _rng.normal(s) * 0.05)(B, S, D)),
            "wqkv": _w((lambda *s: _rng.normal(s) * 0.05)(D, 3 * D)),
            "wo": _w((lambda *s: _rng.normal(s) * 0.05)(D, D)),
        }
    _A_in = _A_setup()

    def _B_setup():
        B, S, D = 1, 2048, 512
        return {
            "x": _w((lambda *s: _rng.normal(s) * 0.05)(B, S, D)),
            "wqkv": _w((lambda *s: _rng.normal(s) * 0.05)(D, 3 * D)),
            "wo": _w((lambda *s: _rng.normal(s) * 0.05)(D, D)),
        }
    _B_in = _B_setup()

    return {
        "A_x": _A_in["x"],
        "A_wqkv": _A_in["wqkv"],
        "A_wo": _A_in["wo"],
        "B_x": _B_in["x"],
        "B_wqkv": _B_in["wqkv"],
        "B_wo": _B_in["wo"],
    }

def reference(A_x, A_wqkv, A_wo, B_x, B_wqkv, B_wo):
    def _A_ref(x, wqkv, wo):
        B, S, D = x.shape
        H = 32; Dh = D // H
        W, dil = 8, 2
        qkv = (lambda x, *d: x.transpose(*d))((x @ wqkv).reshape(B, S, 3, H, Dh), 2, 0, 3, 1, 4)
        q, k, v = qkv[0], qkv[1], qkv[2]
        scale = Dh ** -0.5
        pos = jnp.arange(S)
        off = jnp.arange(W) * dil
        idx = pos[:, None] - off[None, :]
        mask = idx >= 0
        idx_c = jnp.where(mask, idx, 0).reshape(-1)
        kg = k[:, :, idx_c, :].reshape(B, H, S, W, Dh)
        vg = v[:, :, idx_c, :].reshape(B, H, S, W, Dh)
        logits = jnp.einsum("bhsd,bhswd->bhsw", q, kg) * scale
        logits = jnp.where(mask[None, None, :, :], logits, -1e9)
        attn = _softmax(logits, axis=-1)
        o = jnp.einsum("bhsw,bhswd->bhsd", attn, vg)
        return (lambda x, *d: x.transpose(*d))(o, 0, 2, 1, 3).reshape(B, S, D) @ wo

    def _B_ref(x, wqkv, wo):
        B, S, D = x.shape
        H = 32; Dh = D // H
        qkv = (lambda x, *d: x.transpose(*d))((x @ wqkv).reshape(B, S, 3, H, Dh), 2, 0, 3, 1, 4)
        q, k, v = qkv[0], qkv[1], qkv[2]
        scale = Dh ** -0.5
        scores = jnp.einsum("bhqd,bhkd->bhqk", q, k) * scale
        p = _softmax(scores, axis=-1)
        o = jnp.einsum("bhqk,bhkd->bhqd", p, v)
        return (lambda x, *d: x.transpose(*d))(o, 0, 2, 1, 3).reshape(B, S, D) @ wo

    x = A_x
    x = x + _A_ref(_layernorm(x, axis=-1), A_wqkv, A_wo)
    x = x + _B_ref(_layernorm(x, axis=-1), B_wqkv, B_wo)
    x = x + _A_ref(_layernorm(x, axis=-1), A_wqkv, A_wo)
    x = x + _B_ref(_layernorm(x, axis=-1), B_wqkv, B_wo)
    return x
```

```python
import functools
import math

import jax
import jax.numpy as jnp
import numpy as np
from jax import lax
import jax.experimental.pallas as pl
import jax.experimental.pallas.tpu as pltpu

S, D, H, DH = 2048, 512, 32, 16
WIN, DIL = 8, 2
NTILE = S // 128
HALF = NTILE // DIL
NEG = WIN - 1
PITCH = NTILE + 1
EPS = 1e-5
LOG2E = math.log2(math.e)
QSCALE = DH ** -0.5 * LOG2E
MASKED = -1e9 * LOG2E
TB = 512
NQ = 512
CK = 128
NV = 16
KD = 32
HPI = 2
LEAD = 48
PACE0, PACESPAN, PACE_LANE = -80, 120, 384
AHEAD = ((0, 32), (32, CK))
XLU_BLOCKS = 2
FLAGS = {"XLA_TPU_EVENLY_DISTRIBUTE_CRITICAL_NODES": True}
MIN_SUM, MAX_SUM = 2.0 ** -64, 2.0 ** 16

ORDER = [(w[0], int(w[1])) for w in
         "F0 F1 V0 K0 F2 Q0 K1 F3 V1 K2 Q1 K3 V2 B0 S0 Q2 S1 W0 Q3 S2 S3 V3".split()]

f32, bf16 = jnp.float32, jnp.bfloat16


def _token_offset(tile):
    return tile % HALF * DIL + tile // HALF


def _dot(a, b):
    return jnp.dot(a, b, preferred_element_type=f32)


def _project(w_ref, row0, b):
    return _dot(w_ref[pl.ds(row0, D), :], b)


def _dot_nt(a, b):
    return lax.dot_general(a, b, (((1,), (1,)), ((), ())), preferred_element_type=f32)


def _kernel(zero_ref, x_hbm, wqkv_a_hbm, wo_a_hbm, wqkv_b_hbm, wo_b_hbm, out_hbm,
            x_ref, wqkv_a_ref, wo_a_ref, wqkv_b_ref, wo_b_ref, sems, stage, xT, xn, oT, waT, woaT, wbT, wobT, qa, ka, va,
            k_ref, q16, qf, vT, kv, kb, early, sbuf):
    zero = zero_ref[0]

    def set_x(tb, lanes, x):
        xT[tb][:, lanes] = x
        d = x - jnp.sum(x, axis=0, keepdims=True) * (1.0 / D)
        var = jnp.sum(d * d, axis=0, keepdims=True) * (1.0 / D)
        xn[:, pl.ds(tb * TB + lanes.start, lanes.size)] = (d * lax.rsqrt(var + EPS)).astype(bf16)

    pairs = [(x_hbm.at[pl.ds(n * TB, TB)], x_ref.at[pl.ds(n * TB, TB)]) for n in range(S // TB)]
    pairs += [(wqkv_a_hbm, wqkv_a_ref), (wo_a_hbm, wo_a_ref),
              (wqkv_b_hbm, wqkv_b_ref), (wo_b_hbm, wo_b_ref)]
    copies = [pltpu.make_async_copy(src, dst, sems.at[i]) for i, (src, dst) in enumerate(pairs)]
    x_copies, copies = copies[:S // TB], copies[S // TB:]
    for copy in x_copies:
        copy.start()
    for n, copy in enumerate(x_copies):
        copy.wait()
        if n == 0:
            for weights in copies:
                weights.start()
        for i in range(n * TB // NTILE, (n + 1) * TB // NTILE):
            for cb in range(4):
                rows = x_ref[pl.ds(i * NTILE, NTILE), pl.ds(cb * 128, 128)]
                stage[cb, pl.ds(i * PITCH, NTILE), :] = rows.astype(f32)
    row = lax.broadcasted_iota(jnp.int32, (128, 128), 0)
    col = lax.broadcasted_iota(jnp.int32, (128, 128), 1)
    eye = (row == col).astype(f32).astype(bf16)
    for j in range(NTILE):
        tiles = [stage[cb, pl.ds(_token_offset(j), 128, stride=PITCH), :] for cb in range(4)]
        xt = jnp.concatenate([t.T for t in tiles[:XLU_BLOCKS]] +
                             [_dot_nt(eye, t.astype(bf16)) for t in tiles[XLU_BLOCKS:]], axis=0)
        set_x(j * 128 // TB, pl.ds(j * 128 % TB, 128), xt)
    perm = (col == row % 8 * DH + row // 8).astype(f32).astype(bf16)
    copies[0].wait()
    for hg in range(4):
        for part in range(3):
            w = wqkv_a_ref[:, pl.ds(part * D + hg * 128, 128)]
            waT[pl.ds((hg * 3 + part) * 128, 128), :] = _dot_nt(perm, w).astype(bf16)
    copies[1].wait()
    for hg in range(4):
        w = _dot(perm, wo_a_ref[pl.ds(hg * 128, 128), :]).astype(bf16)
        woaT[:, pl.ds(hg * 128, 128)] = w.T
    copies[2].wait()
    copies[3].wait()

    first_values = {}

    def project_a(hg, par):
        g = par * 4 + hg
        lane0 = lax.broadcasted_iota(jnp.int32, (128, 128), 1) == 0
        for tb in range(HALF * 128 // TB):
            r = _dot(waT[pl.ds(hg * 384, 384), :], xn[:, pl.ds(par * HALF * 128 + tb * TB, TB)])
            qa[g][0, :, pl.ds(tb * TB, TB)] = r[:128] * QSCALE
            ka[g][0, :, pl.ds(NEG * 128 + tb * TB, TB)] = r[128:256]
            va[g][0, :, pl.ds(NEG * 128 + tb * TB, TB)] = r[256:]
            if par == 0 and tb == 0:
                first_values[hg] = r[256:, :128]
            for t in range(TB // 128):
                e = tb * (TB // 128) + t - (HALF - NEG)
                if e >= 0:
                    cols = slice(t * 128, t * 128 + 128)
                    ka[g][0, :, pl.ds(e * 128, 128)] = pltpu.roll(r[128:256, cols], 1, 1)
                    va[g][0, :, pl.ds(e * 128, 128)] = jnp.where(
                        lane0, first_values[hg], pltpu.roll(r[256:, cols], 1, 1))

    def attend_a(hg, par):
        g = par * 4 + hg
        lane0 = lax.broadcasted_iota(jnp.int32, (8, 128), 1) == 0
        for j in range(HALF):
            src = [pl.ds((NEG + j - w) * 128, 128) for w in range(WIN)]
            s = [None] * WIN
            for d in range(DH):
                q = qa[g][zero, pl.ds(d * 8, 8), pl.ds(j * 128, 128)]
                for w in range(WIN):
                    t = q * ka[g][zero, pl.ds(d * 8, 8), src[w]]
                    s[w] = t if d == 0 else s[w] + t
            s = [jnp.where(lane0, MASKED, s[w]) if j < w else s[w] for w in range(WIN)]
            m = functools.reduce(jnp.maximum, s)
            p = [jnp.exp2(x - m) for x in s]
            inv = 1.0 / sum(p[1:], p[0])
            p = [x * inv for x in p]
            rows = []
            for d in range(DH):
                o = p[0] * va[g][zero, pl.ds(d * 8, 8), src[0]]
                for w in range(1, WIN):
                    o = o + p[w] * va[g][zero, pl.ds(d * 8, 8), src[w]]
                rows.append(o)
            oT[pl.ds(hg * 128, 128), pl.ds((par * HALF + j) * 128, 128)] = (
                jnp.concatenate(rows, axis=0).astype(bf16))

    def residual_norm(tb, woT):
        x = xT[tb][...] + _project(woT, 0, oT[:, pl.ds(tb * TB, TB)])
        set_x(tb, pl.ds(0, TB), x)

    def squared_norms(rows):
        sq = rows * rows
        return jnp.concatenate(
            [jnp.sum(sq[h * DH:h * DH + 8] + sq[h * DH + 8:(h + 1) * DH], axis=0, keepdims=True)
             for h in range(H)], axis=0)

    def project_k(tb):
        one = (lax.broadcasted_iota(jnp.int32, (KD - DH, 128), 0) == 0).astype(f32).astype(bf16)
        k32 = _project(wbT, D, xn[:, pl.ds(tb * TB, TB)])
        k = k32.astype(bf16)
        for h in range(H):
            for t in range(TB // 128):
                ke = jnp.concatenate([k[h * DH:(h + 1) * DH, t * 128:(t + 1) * 128], one], axis=0).T
                k_ref[h, pl.ds(tb * TB + t * 128, 128), :] = ke
        return squared_norms(k32)

    def project_q(tb):
        cols = pl.ds(tb * TB, TB)
        q = (_project(wbT, 0, xn[:, cols]) * QSCALE).astype(bf16)
        q32 = q.astype(f32)
        qf[:, cols] = q32
        for h in range(H):
            q16[h, pl.ds(0, DH), cols] = q[h * DH:(h + 1) * DH]
        return squared_norms(q32)

    def project_v(tb):
        cols = pl.ds(tb * TB, TB)
        vT[:, cols] = _project(wbT, 2 * D, xn[:, cols])

    def set_shift(tb, q_norms, k_max):
        cols = pl.ds(tb * TB, TB)
        first = lax.broadcasted_iota(jnp.int32, (KD - DH, TB), 0) == 0
        neg_bound = (-jnp.sqrt(q_norms * k_max)).astype(bf16).astype(f32)
        for h in range(H):
            rows = jnp.where(first, neg_bound[h:h + 1], 0.0)
            q16[h, pl.ds(DH, KD - DH), cols] = rows.astype(bf16)

    chunks_per_tile = 128 // NV

    def broadcast_keys(h, kt):
        for d in range(DH):
            t = jnp.broadcast_to(kv[h, d:d + 1, pl.ds(kt * 128, 128)], (128, 128)).T
            for c in range(chunks_per_tile):
                kb[kt * chunks_per_tile + c, d] = t[c * NV:(c + 1) * NV]

    nchunk, mrows = S // CK, CK - NV

    def weights_ahead(h, r0, r1):
        s = _dot(k_ref[h, pl.ds(r0, r1 - r0), :], q16[h, :, pl.ds(0, NQ)])
        early[pl.ds(r0, r1 - r0), :] = jnp.exp2(s)

    def attend_b(it, ok):
        steps = [(u, q0, c) for u in range(HPI) for q0 in range(0, S, NQ) for c in range(nchunk)]
        stream = [(i, r) for i in range(1, len(steps)) for r in range(0, mrows, 16)]
        never = jnp.full((8, 128), zero_ref[0], jnp.int32) != 0
        scores, cache = {}, {}
        following = jnp.minimum((it + 1) * HPI, H - 1)

        def issue(g0, g1):
            while g0 < g1:
                u, q0, _ = steps[stream[g0][0]]
                g = g0
                while g < g1 and steps[stream[g][0]][:2] == (u, q0):
                    g += 1
                h = it * HPI + u
                keys = [k_ref[h, pl.ds(steps[i][2] * CK + r, 16), :] for i, r in stream[g0:g]]
                s = _dot(jnp.concatenate(keys, axis=0), q16[h, :, pl.ds(q0, NQ)])
                for n, e in enumerate(stream[g0:g]):
                    scores[e] = s[n * 16:(n + 1) * 16]
                g0 = g

        def vpu_keys(i, d):
            u, _, c = steps[i]
            if u == 0:
                kd = kb[c, d]
            else:
                kt = c // chunks_per_tile
                if ('k', u, d, kt) not in cache:
                    row = kv[it * HPI + u, d:d + 1, pl.ds(kt * 128, 128)]
                    cache['k', u, d, kt] = jnp.broadcast_to(row, (128, 128)).T
                r = c % chunks_per_tile * NV
                kd = cache['k', u, d, kt][r:r + NV]
            g = ((i - 1) * mrows + PACE0 + d * PACESPAN // DH) // 8
            if g < 0:
                pace = jnp.zeros((8, 128), f32)
            else:
                pace = scores[stream[g // 2]][g % 2 * 8:g % 2 * 8 + 8, PACE_LANE:PACE_LANE + 128]
            return jnp.concatenate(
                [jnp.where(never, pace, kd[r:r + 8]) for r in range(0, NV, 8)], axis=0)

        def vpu_scores(i):
            u, q0, _ = steps[i]
            h = it * HPI + u
            qh = qf.at[pl.ds(pl.multiple_of(h * DH, DH), DH)]
            keys, out = {}, []
            for t in range(NQ // 128):
                cols = pl.ds(q0 + t * 128, 128)
                if (u, q0, t) not in cache:
                    cache[u, q0, t] = q16[h, pl.ds(DH, KD - DH), cols].astype(f32)[:1]
                for d in range(DH):
                    if d not in keys:
                        keys[d] = vpu_keys(i, d)
                    x = keys[d] * qh[d:d + 1, cols]
                    a = x + cache[u, q0, t] if d == 0 else a + x
                out.append(a)
            return jnp.concatenate(out, axis=1)

        pos = 0
        for i, (u, q0, c) in enumerate(steps):
            h = it * HPI + u
            end = min(len(stream), ((i + 1) * mrows + LEAD) // 16)
            issue(pos, end)
            pos = end
            if i >= len(steps) - 2:
                weights_ahead(following, *AHEAD[i - len(steps) + 2])
            if i == 0:
                p = early[...]
            else:
                s = [scores[i, r] for r in range(0, mrows, 16)] + [vpu_scores(i)]
                p = jnp.exp2(jnp.concatenate(s, axis=0))
            part = jnp.sum(p.reshape(CK // 8, 8, NQ), axis=0)
            den = part if c == 0 else den + part
            rows = pl.ds(pl.multiple_of(h * DH, DH), DH)
            o = _dot(vT[rows, pl.ds(c * CK, CK)], p)
            acc = o if c == 0 else acc + o
            if i >= len(steps) - nchunk and (c + 1) % chunks_per_tile == 0:
                broadcast_keys(following, c // chunks_per_tile)
            if c == nchunk - 1:
                total = jnp.sum(den, axis=0, keepdims=True)
                ok = jnp.where((total >= MIN_SUM) & (total <= MAX_SUM), ok, 0.0)
                oT[rows, pl.ds(q0, NQ)] = (acc / total).astype(bf16)
        return ok

    def attend_b_true_max(i, _):
        h, qb = i // (S // NQ), i % (S // NQ)
        rows = pl.ds(pl.multiple_of(h * DH, DH), DH)
        cols = pl.ds(pl.multiple_of(qb * NQ, NQ), NQ)
        w = jnp.concatenate([q16[h, pl.ds(0, DH), cols], jnp.zeros((KD - DH, NQ), bf16)], axis=0)

        def scores(c, m):
            keys = pl.ds(pl.multiple_of(c * 256, 256), 256)
            s = _dot(k_ref[h, keys, :], w)
            sbuf[keys, :] = s
            return jnp.maximum(m, jnp.max(s, axis=0, keepdims=True))

        m = lax.fori_loop(0, S // 256, scores, jnp.full((1, NQ), -jnp.inf, f32))

        def weigh(c, carry):
            keys = pl.ds(pl.multiple_of(c * 256, 256), 256)
            p = jnp.exp2(sbuf[keys, :] - m)
            return carry[0] + _dot(vT[rows, keys], p), carry[1] + jnp.sum(p, axis=0, keepdims=True)

        acc, total = lax.fori_loop(
            0, S // 256, weigh, (jnp.zeros((DH, NQ), f32), jnp.zeros((1, NQ), f32)))
        oT[rows, cols] = (acc / total).astype(bf16)

    def layer_pair(rep, carry):
        for nb in range(3 * D // 128):
            wbT[pl.ds(nb * 128, 128), :] = wqkv_b_ref[:, pl.ds(nb * 128, 128)].T
        for nb in range(D // 128):
            wobT[pl.ds(nb * 128, 128), :] = wo_b_ref[:, pl.ds(nb * 128, 128)].T
        for par in range(DIL):
            for hg in range(4):
                project_a(hg, par)
                attend_a(hg, par)
        k_norms, q_norms = [], []
        for op, tb in ORDER:
            if op == "F":
                residual_norm(tb, woaT)
            elif op == "K":
                k_norms.append(project_k(tb))
            elif op == "Q":
                q_norms.append(project_q(tb))
            elif op == "V":
                project_v(tb)
            elif op == "B":
                k_max = jnp.max(functools.reduce(jnp.maximum, k_norms), axis=1, keepdims=True)
                for h in range(H):
                    keys = [k_ref[h + zero, pl.ds(c * CK + mrows, NV), :] for c in range(nchunk)]
                    kv[h] = jnp.concatenate(keys, axis=0).astype(f32).T
                for kt in range(S // CK // chunks_per_tile):
                    broadcast_keys(0, kt)
            elif op == "S":
                set_shift(tb, q_norms[tb], k_max)
            else:
                weights_ahead(0, 0, CK)
        ok = lax.fori_loop(0, H // HPI, attend_b, jnp.ones((1, NQ), f32))

        @pl.when(jnp.min(ok) < 1.0)
        def _():
            lax.fori_loop(0, H * (S // NQ), attend_b_true_max, None)

        @pl.when(rep == 0)
        def _():
            for tb in range(S // TB):
                residual_norm(tb, wobT)
        return carry

    lax.fori_loop(0, 2, layer_pair, None)

    stores = []
    for cb in range(4):
        feats = pl.ds(cb * 128, 128)
        for tb in range(S // TB):
            cols = pl.ds(tb * TB, TB)
            x = xT[tb][feats, :] + _dot(wobT[feats, :], oT[:, cols])
            for t in range(TB // 128):
                j = tb * (TB // 128) + t
                stage[cb, pl.ds(_token_offset(j), 128, stride=PITCH), :] = x[:, t * 128:(t + 1) * 128].T
        for half in range(2):
            for i in range(half * 64, half * 64 + 64):
                rows = stage[cb, pl.ds(i * PITCH, NTILE), :]
                x_ref[pl.ds(i * NTILE, NTILE), feats] = rows.astype(x_ref.dtype)
            part = (pl.ds(half * S // 2, S // 2), feats)
            stores.append(pltpu.make_async_copy(
                x_ref.at[part], out_hbm.at[part], sems.at[cb * 2 + half]))
            stores[-1].start()
    for store in stores:
        store.wait()


@jax.jit
def pallas_interleave_layers__sliding_local_dilated__softmax_full_mha__prompt_kernel(
    A_x: jax.Array,
    A_wqkv: jax.Array,
    A_wo: jax.Array,
    B_x: jax.Array,
    B_wqkv: jax.Array,
    B_wo: jax.Array,
):
    del B_x
    assert A_x.dtype == bf16 and A_wqkv.dtype == bf16 and A_wo.dtype == bf16
    hbm = pl.BlockSpec(memory_space=pl.ANY)
    hist = (NEG + HALF) * 128
    nvpu = S // CK * NV
    out = pl.pallas_call(
        _kernel,
        out_shape=jax.ShapeDtypeStruct((S, D), A_x.dtype),
        in_specs=[pl.BlockSpec(memory_space=pltpu.SMEM)] + [hbm] * 5,
        out_specs=hbm,
        scratch_shapes=[
            pltpu.VMEM((S, D), A_x.dtype),
            pltpu.VMEM(A_wqkv.shape, A_wqkv.dtype),
            pltpu.VMEM(A_wo.shape, A_wo.dtype),
            pltpu.VMEM(B_wqkv.shape, B_wqkv.dtype),
            pltpu.VMEM(B_wo.shape, B_wo.dtype),
            pltpu.SemaphoreType.DMA((8,)),
            pltpu.VMEM((4, 129 * PITCH + 7, 128), f32),
            [pltpu.VMEM((D, TB), f32)] * (S // TB),
            pltpu.VMEM((D, S), bf16),
            pltpu.VMEM((D, S), bf16),
            pltpu.VMEM((3 * D, D), bf16),
            pltpu.VMEM((D, D), bf16),
            pltpu.VMEM((3 * D, D), bf16),
            pltpu.VMEM((D, D), bf16),
            [pltpu.VMEM((1, 128, HALF * 128), f32)] * 8,
            [pltpu.VMEM((1, 128, hist), f32)] * 8,
            [pltpu.VMEM((1, 128, hist), f32)] * 8,
            pltpu.VMEM((H, S, KD), bf16),
            pltpu.VMEM((H, KD, S), bf16),
            pltpu.VMEM((D, S), f32),
            pltpu.VMEM((D, S), f32),
            pltpu.VMEM((H, KD, nvpu), f32),
            pltpu.VMEM((S // CK, DH, NV, 128), f32),
            pltpu.VMEM((CK, NQ), f32),
            pltpu.VMEM((S, NQ), f32),
        ],
        compiler_params=pltpu.CompilerParams(vmem_limit_bytes=100 * 2 ** 20, flags=FLAGS),
    )(np.zeros((1,), np.int32), A_x.reshape(S, D), A_wqkv, A_wo, B_wqkv, B_wo)
    return out.reshape(A_x.shape)
```
